```python
import os as _os
_os.environ.setdefault("JAX_PLATFORMS", "cpu")
import jax
import jax.numpy as jnp

def _softmax(x, axis=-1):
    return jax.nn.softmax(x, axis=axis)
def _gelu(x):
    return jax.nn.gelu(x, approximate=True)
def _silu(x):
    return jax.nn.silu(x)
def _sigmoid(x):
    return jax.nn.sigmoid(x)
def _layernorm(x, axis=-1, eps=1e-5):
    m = jnp.mean(x, axis=axis, keepdims=True)
    v = jnp.var(x, axis=axis, keepdims=True)
    return (x - m) / jnp.sqrt(v + eps)
def _scatter_add(tgt, idx, src, axis=0):
    return tgt.at[idx].add(src)
def _segment_sum(src, seg, n):
    return jax.ops.segment_sum(src, seg, n)
class _Rng:
    def __init__(self, key):
        self._k = key
    def _next(self):
        self._k, sub = jax.random.split(self._k)
        return sub
    def normal(self, shape):
        return jax.random.normal(self._next(), shape, dtype=jnp.bfloat16)
    def randint(self, lo, hi, shape):
        return jax.random.randint(self._next(), shape, lo, hi, dtype=jnp.int32)
    def uniform(self, shape, lo=0.0, hi=1.0):
        return jax.random.uniform(self._next(), shape, jnp.bfloat16, lo, hi)
    def permutation(self, n):
        return jax.random.permutation(self._next(), n)


kernel_name = 'recurrent_scan__ssm_conv_s5__mixer_s_mlp__prompt'

def setup_inputs():
    _rng = _Rng(jax.random.key(int.from_bytes(__import__("os").urandom(4), "little")))
    _w = (lambda a: (lambda t: t.astype(jnp.bfloat16) if jnp.issubdtype(t.dtype, jnp.floating) else t)(jnp.asarray(a)))
    def _A_setup():
        B, S, D = 1, 2048, 640
        P = D
        Lambda_re = -0.5 * jnp.exp((lambda *s: _rng.normal(s) * 0.8)(P))
        Lambda_im = (lambda *s: _rng.normal(s) * 0.8)(P) * 1.0
        B_re = (lambda *s: _rng.normal(s) * 0.8)(P, D) * (D ** -0.5)
        B_im = (lambda *s: _rng.normal(s) * 0.8)(P, D) * (D ** -0.5)
        C_re = (lambda *s: _rng.normal(s) * 0.8)(D, P) * (P ** -0.5)
        C_im = (lambda *s: _rng.normal(s) * 0.8)(D, P) * (P ** -0.5)
        log_dt = (lambda *s: _rng.normal(s) * 0.8)(P) * 0.3 - 2.0
        Dskip = (lambda *s: _rng.normal(s) * 0.8)(D)
        return {
            "x": _w((lambda *s: _rng.normal(s) * 0.05)(B, S, D)),
            "Lambda_re": _w(Lambda_re),
            "Lambda_im": _w(Lambda_im),
            "B_re": _w(B_re),
            "B_im": _w(B_im),
            "C_re": _w(C_re),
            "C_im": _w(C_im),
            "log_dt": _w(log_dt),
            "Dskip": _w(Dskip),
        }
    _A_in = _A_setup()

    def _B_setup():
        B, S, D, F = 1, 2048, 640, 1536
        return {
            "x":  _w((lambda *s: _rng.normal(s) * 0.05)(B, S, D)),
            "w1": _w((lambda *s: _rng.normal(s) * 0.8)(D, D) * (D ** -0.5)),
            "w2": _w((lambda *s: _rng.normal(s) * 0.8)(D, D) * (D ** -0.5)),
            "w3": _w((lambda *s: _rng.normal(s) * 0.8)(D, F) * (D ** -0.5)),
            "w4": _w((lambda *s: _rng.normal(s) * 0.8)(F, D) * (F ** -0.5)),
        }
    _B_in = _B_setup()

    return {
        "A_x": _A_in["x"],
        "A_Lambda_re": _A_in["Lambda_re"],
        "A_Lambda_im": _A_in["Lambda_im"],
        "A_B_re": _A_in["B_re"],
        "A_B_im": _A_in["B_im"],
        "A_C_re": _A_in["C_re"],
        "A_C_im": _A_in["C_im"],
        "A_log_dt": _A_in["log_dt"],
        "A_Dskip": _A_in["Dskip"],
        "B_x": _B_in["x"],
        "B_w1": _B_in["w1"],
        "B_w2": _B_in["w2"],
        "B_w3": _B_in["w3"],
        "B_w4": _B_in["w4"],
    }

def reference(A_x, A_Lambda_re, A_Lambda_im, A_B_re, A_B_im, A_C_re, A_C_im, A_log_dt, A_Dskip, B_x, B_w1, B_w2, B_w3, B_w4):
    def _A_ref(x, Lambda_re, Lambda_im, B_re, B_im, C_re, C_im, log_dt, Dskip):
        Bsz, L, H = x.shape
        Lam = Lambda_re + 1j * Lambda_im
        Bmat = B_re + 1j * B_im
        Cmat = C_re + 1j * C_im
        dt = jnp.exp(log_dt)
        Lam_bar = jnp.exp(dt * Lam)
        B_bar = ((Lam_bar - 1.0) / Lam)[:, None] * Bmat
        Bu = jnp.einsum("bld,pd->blp", x + 0j, B_bar)
        h = jnp.zeros_like(Bu[:, 0, :])
        hs = []
        for t in range(L):
            h = Lam_bar[None, :] * h + Bu[:, t, :]
            hs.append(h)
        hseq = jnp.stack(hs, 1)
        y = 2.0 * jnp.einsum("blp,dp->bld", hseq, Cmat).real + x * Dskip[None, None, :]
        return y

    def _B_ref(x, w1, w2, w3, w4):
        B, S, D = x.shape
        h = _gelu(_layernorm(x, axis=-1) @ w1)
        c = D // 4
        g0 = jnp.pad(h[:, :, 0*c:1*c], ((0, 0), (1, 0), (0, 0)))[:, :S, :]
        g1 = jnp.pad(h[:, :, 1*c:2*c], ((0, 0), (0, 1), (0, 0)))[:, 1:, :]
        g2 = jnp.pad(h[:, :, 2*c:3*c], ((0, 0), (2, 0), (0, 0)))[:, :S, :]
        g3 = jnp.pad(h[:, :, 3*c:   ], ((0, 0), (0, 2), (0, 0)))[:, 2:, :]
        hs = jnp.concatenate([g0, g1, g2, g3], axis=-1) @ w2
        x1 = x + hs
        h2 = _gelu(_layernorm(x1, axis=-1) @ w3) @ w4
        return x1 + h2

    x = A_x
    xn = _layernorm(x, axis=-1)
    s = _A_ref(xn, A_Lambda_re, A_Lambda_im, A_B_re, A_B_im, A_C_re, A_C_im, A_log_dt, A_Dskip)
    g = _silu(_B_ref(xn, B_w1, B_w2, B_w3, B_w4))
    return x + s * g
```

```python
import jax
import jax.numpy as jnp
import jax.experimental.pallas as pl
import jax.experimental.pallas.tpu as pltpu

L = 2048
D = 640
P = 640
F = 1536
TM = 256
NC = L // TM
LANES = 128
NT = D // LANES
EPS = 1e-5
PAD = 8

_NT_DIMS = (((1,), (1,)), ((), ()))


def _layernorm(v):
    m = jnp.mean(v, axis=-1, keepdims=True)
    c = v - m
    var = jnp.mean(c * c, axis=-1, keepdims=True)
    return c * jax.lax.rsqrt(var + EPS)


def _gelu(v):
    k0 = 0.7978845608028654
    k1 = 0.044715 * k0
    inner = v * (k0 + k1 * (v * v))
    return (0.5 * v) * (1.0 + jnp.tanh(inner))


def _silu(v):
    return v * (0.5 + 0.5 * jnp.tanh(0.5 * v))


def _kernel(x_hbm, lre_ref, lim_ref, bre_hbm, bim_hbm, cre_hbm, cim_hbm, ldt_ref, dsk_ref,
            w1_hbm, w2_hbm, w3_hbm, w4_hbm, o_hbm,
            x_v, bre_v, bim_v, cre_v, cim_v, w1_v, w2_v, w3_v, w4_v,
            xn_v, h1_v, y_v, o_v, tab_v, carry_v, xsem, wsem, osem):
    def x_copy(k):
        return pltpu.make_async_copy(x_hbm.at[pl.ds(k * TM, TM), :], x_v.at[pl.ds(k * TM, TM), :], xsem.at[k])

    wpairs = [(w1_hbm, w1_v), (bre_hbm, bre_v), (bim_hbm, bim_v), (cre_hbm, cre_v), (cim_hbm, cim_v),
              (w2_hbm, w2_v), (w3_hbm, w3_v), (w4_hbm, w4_v)]
    wcopies = [pltpu.make_async_copy(s, d, wsem.at[i]) for i, (s, d) in enumerate(wpairs)]
    x_copy(0).start()
    for c in wcopies[:5]:
        c.start()
    for k in range(1, NC):
        x_copy(k).start()
    for c in wcopies[5:]:
        c.start()

    lre = lre_ref[...].astype(jnp.float32).reshape(1, P)
    lim = lim_ref[...].astype(jnp.float32).reshape(1, P)
    dt = jnp.exp(ldt_ref[...].astype(jnp.float32)).astype(jnp.bfloat16).astype(jnp.float32).reshape(1, P)
    zr = dt * lre
    zi = dt * lim
    mag = jnp.exp(zr)
    ar = mag * jnp.cos(zi)
    ai = mag * jnp.sin(zi)
    den = 2.0 / (lre * lre + lim * lim)
    nr = ar - 1.0
    fr = (nr * lre + ai * lim) * den
    fi = (ai * lre - nr * lim) * den
    ai = -ai
    def cmul(a, b):
        return a[0] * b[0] - a[1] * b[1], a[0] * b[1] + a[1] * b[0]
    p1 = (ar, ai)
    p2 = cmul(p1, p1)
    p3 = cmul(p2, p1)
    p4 = cmul(p2, p2)
    p5 = cmul(p4, p1)
    p6 = cmul(p4, p2)
    p7 = cmul(p4, p3)
    p8 = cmul(p4, p4)
    sub = jax.lax.broadcasted_iota(jnp.int32, (8, P), 0)
    for i, (d, p) in enumerate(((1, p1), (2, p2), (4, p4))):
        tab_v[2 * i] = jnp.where(sub >= d, jnp.broadcast_to(p[0], (8, P)), 0.0)
        tab_v[2 * i + 1] = jnp.where(sub >= d, jnp.broadcast_to(p[1], (8, P)), 0.0)
    pr = jnp.broadcast_to(p1[0], (8, P))
    pi = jnp.broadcast_to(p1[1], (8, P))
    for d, p in enumerate((p2, p3, p4, p5, p6, p7, p8), start=1):
        pr = jnp.where(sub >= d, jnp.broadcast_to(p[0], (8, P)), pr)
        pi = jnp.where(sub >= d, jnp.broadcast_to(p[1], (8, P)), pi)
    tab_v[6] = pr
    tab_v[7] = pi
    tab_v[8] = jnp.broadcast_to(fr, (8, P))
    tab_v[9] = jnp.broadcast_to(fi, (8, P))
    tab_v[10] = jnp.broadcast_to(dsk_ref[...].astype(jnp.float32).reshape(1, P), (8, P))
    carry_v[...] = jnp.zeros_like(carry_v)
    h1_v[0:PAD, :] = jnp.zeros((PAD, D), jnp.float32)
    h1_v[PAD + L:PAD + L + PAD, :] = jnp.zeros((PAD, D), jnp.float32)

    G = TM // 8

    def phase1(k, first):
        r0 = 0 if first else pl.multiple_of(k * TM, TM)
        rows = pl.ds(r0, TM)
        x_copy(k).wait()
        x = x_v[rows, :].astype(jnp.float32)
        xn = _layernorm(x).astype(jnp.bfloat16)
        xn_v[rows, :] = xn
        xn2 = _layernorm(xn.astype(jnp.float32)).astype(jnp.bfloat16)
        if first:
            wcopies[0].wait()
        h1 = _gelu(jnp.dot(xn2, w1_v[...], preferred_element_type=jnp.float32))
        h1_v[pl.ds(pl.multiple_of(r0 + PAD, 8), TM), :] = h1
        if first:
            wcopies[1].wait()
            wcopies[2].wait()
        ur = jax.lax.dot_general(xn, bre_v[...], _NT_DIMS, preferred_element_type=jnp.float32)
        ui = jax.lax.dot_general(xn, bim_v[...], _NT_DIMS, preferred_element_type=jnp.float32)
        hrs, his = [], []
        for j in range(NT):
            ls = slice(j * LANES, (j + 1) * LANES)
            u_r = ur[:, ls].reshape(G, 8, LANES)
            u_i = ui[:, ls].reshape(G, 8, LANES)
            f_r = tab_v[8, :, ls]
            f_i = tab_v[9, :, ls]
            hr = f_r * u_r - f_i * u_i
            hi = -(f_r * u_i + f_i * u_r)
            for i, d in enumerate((1, 2, 4)):
                a_r = tab_v[2 * i, :, ls]
                a_i = tab_v[2 * i + 1, :, ls]
                sr = pltpu.roll(hr, d, 1)
                si = pltpu.roll(hi, d, 1)
                hr, hi = hr + (a_r * sr - a_i * si), hi + (a_r * si + a_i * sr)
            q_r = tab_v[6, :, ls]
            q_i = tab_v[7, :, ls]
            c_r = carry_v[0, :, ls]
            c_i = carry_v[1, :, ls]
            outr, outi = [], []
            for g in range(G):
                gr = hr[g] + (q_r * c_r - q_i * c_i)
                gi = hi[g] + (q_r * c_i + q_i * c_r)
                outr.append(gr)
                outi.append(gi)
                c_r = jnp.broadcast_to(gr[7:8, :], (8, LANES))
                c_i = jnp.broadcast_to(gi[7:8, :], (8, LANES))
            carry_v[0, :, ls] = c_r
            carry_v[1, :, ls] = c_i
            hrs.append(jnp.concatenate(outr, axis=0).astype(jnp.bfloat16))
            his.append(jnp.concatenate(outi, axis=0).astype(jnp.bfloat16))
        h_r = jnp.concatenate(hrs, axis=1)
        h_i = jnp.concatenate(his, axis=1)
        if first:
            wcopies[3].wait()
            wcopies[4].wait()
        y = jax.lax.dot_general(h_r, cre_v[...], _NT_DIMS, preferred_element_type=jnp.float32)
        y = y + jax.lax.dot_general(h_i, cim_v[...], _NT_DIMS, preferred_element_type=jnp.float32)
        y_v[rows, :] = y + xn.astype(jnp.float32) * tab_v[10, 0:1, :]

    phase1(0, True)

    def p1_body(k, c):
        phase1(k, False)
        return c
    jax.lax.fori_loop(1, NC, p1_body, 0)

    for c in wcopies[5:]:
        c.wait()

    def o_copy(k):
        return pltpu.make_async_copy(o_v.at[pl.ds(k * TM, TM), :], o_hbm.at[pl.ds(k * TM, TM), :], osem.at[k])

    lane = jax.lax.broadcasted_iota(jnp.int32, (TM, LANES), 1)

    def p2_body(k, c):
        r0 = pl.multiple_of(k * TM, TM)
        rows = pl.ds(r0, TM)

        def sh(j, s):
            win = h1_v[pl.ds(r0, TM + 2 * PAD), j * LANES:(j + 1) * LANES]
            return win[PAD - s:PAD - s + TM]
        g = jnp.concatenate([
            sh(0, 1),
            jnp.where(lane < 32, sh(1, 1), sh(1, -1)),
            jnp.where(lane < 64, sh(2, -1), sh(2, 2)),
            jnp.where(lane < 96, sh(3, 2), sh(3, -2)),
            sh(4, -2)], axis=1).astype(jnp.bfloat16)
        hs = jnp.dot(g, w2_v[...], preferred_element_type=jnp.float32)
        x1 = xn_v[rows, :].astype(jnp.float32) + hs
        xn3 = _layernorm(x1).astype(jnp.bfloat16)
        hid = _gelu(jnp.dot(xn3, w3_v[...], preferred_element_type=jnp.float32)).astype(jnp.bfloat16)
        h2 = jnp.dot(hid, w4_v[...], preferred_element_type=jnp.float32)
        gate = _silu(x1 + h2)
        o_v[rows, :] = x_v[rows, :].astype(jnp.float32) + y_v[rows, :] * gate
        o_copy(k).start()
        return c
    jax.lax.fori_loop(0, NC, p2_body, 0)
    for k in range(NC):
        o_copy(k).wait()


@jax.jit
def pallas_recurrent_scan__ssm_conv_s5__mixer_s_mlp__prompt_kernel(
    A_x: jax.Array,
    A_Lambda_re: jax.Array,
    A_Lambda_im: jax.Array,
    A_B_re: jax.Array,
    A_B_im: jax.Array,
    A_C_re: jax.Array,
    A_C_im: jax.Array,
    A_log_dt: jax.Array,
    A_Dskip: jax.Array,
    B_x: jax.Array,
    B_w1: jax.Array,
    B_w2: jax.Array,
    B_w3: jax.Array,
    B_w4: jax.Array,
):
    del B_x
    x = A_x.reshape(L, D)
    hbm = pl.BlockSpec(memory_space=pl.ANY)
    vmem = pl.BlockSpec(memory_space=pltpu.VMEM)
    bf = jnp.bfloat16
    out = pl.pallas_call(
        _kernel,
        out_shape=jax.ShapeDtypeStruct((L, D), jnp.float32),
        in_specs=[hbm, vmem, vmem, hbm, hbm, hbm, hbm, vmem, vmem, hbm, hbm, hbm, hbm],
        out_specs=hbm,
        scratch_shapes=[
            pltpu.VMEM((L, D), bf),
            pltpu.VMEM((P, D), bf), pltpu.VMEM((P, D), bf),
            pltpu.VMEM((D, P), bf), pltpu.VMEM((D, P), bf),
            pltpu.VMEM((D, D), bf), pltpu.VMEM((D, D), bf),
            pltpu.VMEM((D, F), bf), pltpu.VMEM((F, D), bf),
            pltpu.VMEM((L, D), bf),
            pltpu.VMEM((L + 2 * PAD, D), jnp.float32),
            pltpu.VMEM((L, D), jnp.float32),
            pltpu.VMEM((L, D), jnp.float32),
            pltpu.VMEM((11, 8, P), jnp.float32),
            pltpu.VMEM((2, 8, P), jnp.float32),
            pltpu.SemaphoreType.DMA((NC,)),
            pltpu.SemaphoreType.DMA((8,)),
            pltpu.SemaphoreType.DMA((NC,)),
        ],
        compiler_params=pltpu.CompilerParams(vmem_limit_bytes=100 * 1024 * 1024),
    )(x, A_Lambda_re, A_Lambda_im, A_B_re, A_B_im, A_C_re, A_C_im, A_log_dt, A_Dskip,
      B_w1, B_w2, B_w3, B_w4)
    return out.reshape(1, L, D)
```

```python
import jax
import jax.numpy as jnp
import jax.experimental.pallas as pl
import jax.experimental.pallas.tpu as pltpu

L = 2048
D = 640
P = 640
F = 1536
TM = 256
NC = L // TM
LANES = 128
NT = D // LANES
EPS = 1e-5
PAD = 8
LN_RB = 16
NSLOT = 3
SEG = TM // 8
NA = 3
ORDER = [("w", 0), ("w", 1), ("w", 2), ("w", 3), ("w", 4), ("c", 0), ("c", 1),
         ("b", 0), ("b", 1), ("b", 2), ("b", 3), ("b", 4), ("c", 2), ("c", 3), ("c", 4)]

_NT_DIMS = (((1,), (1,)), ((), ()))
f32 = jnp.float32
bf16 = jnp.bfloat16
u32 = jnp.uint32


def _layernorm(v):
    m = jnp.mean(v, axis=-1, keepdims=True)
    c = v - m
    var = jnp.mean(c * c, axis=-1, keepdims=True)
    return c * jax.lax.rsqrt(var + EPS)


def _gelu(v):
    k0 = 0.7978845608028654
    k1 = 0.044715 * k0
    inner = v * (k0 + k1 * (v * v))
    return (0.5 * v) * (1.0 + jnp.tanh(inner))


def _silu(v):
    return v * (0.5 + 0.5 * jnp.tanh(0.5 * v))


def _pk(v):
    return pltpu.bitcast(v, u32)


def _upk(v):
    return pltpu.bitcast(v, bf16)


def _kernel(x_hbm, lre_hbm, lim_hbm, bre_hbm, bim_hbm, cre_hbm, cim_hbm, ldt_hbm, dsk_hbm,
            w1_hbm, w2_hbm, w3_hbm, w4_hbm, o_hbm,
            x_v, bre_v, bim_v, cre_v, cim_v, w1_v, w2_v, w3_v, w4_v,
            xn_v, h1_v, y_v, o_v,
            hra, hia, hrb, hib, x1a, x1b, n3a, n3b,
            tab_v, carry_v, lre_ref, lim_ref, ldt_ref, dsk_ref, xsem, wsem, osem, ssem, *extra):
    u_ab = (extra[:2 * NT], extra[2 * NT:4 * NT])
    lna, lnb = extra[4 * NT:4 * NT + 2], extra[4 * NT + 2:4 * NT + 4]
    lnt_v = extra[4 * NT + 4]
    hc, lnc = extra[4 * NT + 5:4 * NT + 7], extra[4 * NT + 7:4 * NT + 9]
    pk, upk = _pk, _upk

    def rows_of(k, n=TM, off=0):
        if isinstance(k, int):
            return pl.ds(k * TM + off, n)
        return pl.ds(pl.multiple_of(k * TM + off, 8), n)

    def prow(k, n=TM // 2, off=0):
        if isinstance(k, int):
            return pl.ds(k * (TM // 2) + off, n)
        return pl.ds(pl.multiple_of(k * (TM // 2) + off, 8), n)

    def tile(j):
        return slice(j * LANES, (j + 1) * LANES)

    def x_copy(k):
        return pltpu.make_async_copy(x_hbm.bitcast(u32).at[prow(k), :], x_v.at[prow(k), :], xsem.at[k])

    wpairs = dict(bim=(bim_hbm, bim_v), w1=(w1_hbm, w1_v), cre=(cre_hbm, cre_v),
                  cim=(cim_hbm, cim_v), w2=(w2_hbm, w2_v), w3=(w3_hbm, w3_v), w4=(w4_hbm, w4_v))
    wc = {n: pltpu.make_async_copy(s.bitcast(u32), d, wsem.at[i + 1])
          for i, (n, (s, d)) in enumerate(wpairs.items())}
    bre_a = pltpu.make_async_copy(bre_hbm.bitcast(u32).at[0:64 * NA, :], bre_v.at[0:64 * NA, :], wsem.at[0])
    bre_b = pltpu.make_async_copy(bre_hbm.bitcast(u32).at[64 * NA:, :], bre_v.at[64 * NA:, :], wsem.at[8])
    small = [pltpu.make_async_copy(s, d, ssem.at[i]) for i, (s, d) in enumerate(
        ((lre_hbm, lre_ref), (lim_hbm, lim_ref), (ldt_hbm, ldt_ref), (dsk_hbm, dsk_ref)))]
    for c in small:
        c.start()
    x_copy(0).start()
    bre_a.start()
    x_copy(1).start()
    bre_b.start()
    wc["bim"].start()
    wc["w1"].start()
    wc["cre"].start()
    wc["cim"].start()
    for k in range(2, NC):
        x_copy(k).start()
    wc["w2"].start()
    wc["w3"].start()
    wc["w4"].start()
    for c in small:
        c.wait()

    lre = lre_ref[...].astype(f32).reshape(1, P)
    lim = lim_ref[...].astype(f32).reshape(1, P)
    dt = jnp.exp(ldt_ref[...].astype(f32)).astype(bf16).astype(f32).reshape(1, P)
    zr = dt * lre
    zi = dt * lim
    mag = jnp.exp(zr)
    ar = mag * jnp.cos(zi)
    ai = mag * jnp.sin(zi)
    den = 2.0 / (lre * lre + lim * lim)
    nr = ar - 1.0
    fr = (nr * lre + ai * lim) * den
    fi = (ai * lre - nr * lim) * den

    def cmul(a, b):
        return a[0] * b[0] - a[1] * b[1], a[0] * b[1] + a[1] * b[0]

    def bc(v):
        return jnp.broadcast_to(v, (8, P))
    seg = (ar, ai)
    for _ in range(SEG.bit_length() - 1):
        seg = cmul(seg, seg)
    s1 = seg
    s2 = cmul(s1, s1)
    s3 = cmul(s2, s1)
    s4 = cmul(s2, s2)
    s5 = cmul(s4, s1)
    s6 = cmul(s4, s2)
    s7 = cmul(s4, s3)
    s8 = cmul(s4, s4)
    sub = jax.lax.broadcasted_iota(jnp.int32, (8, P), 0)
    for i, (d, p) in enumerate(((1, s1), (2, s2), (4, s4))):
        tab_v[2 * i] = jnp.where(sub >= d, bc(p[0]), 0.0)
        tab_v[2 * i + 1] = jnp.where(sub >= d, bc(p[1]), 0.0)
    pr, pi = bc(s1[0]), bc(s1[1])
    for d, p in enumerate((s2, s3, s4, s5, s6, s7, s8), start=1):
        pr = jnp.where(sub >= d, bc(p[0]), pr)
        pi = jnp.where(sub >= d, bc(p[1]), pi)
    tab_v[6] = pr
    tab_v[7] = pi
    tab_v[8] = bc(fr)
    tab_v[9] = bc(fi)
    tab_v[10] = bc(dsk_ref[...].astype(f32).reshape(1, P))
    tab_v[11] = bc(ar)
    tab_v[12] = bc(ai)
    carry_v[...] = jnp.zeros_like(carry_v)
    lnt_v[...] = jnp.zeros_like(lnt_v)
    h1_v[0:PAD, :] = jnp.zeros((PAD, D), f32)
    h1_v[PAD + L:PAD + L + PAD, :] = jnp.zeros((PAD, D), f32)

    def ln_slot(v, slot):
        t = lnt_v.at[slot]
        c = v - jnp.mean(v, axis=-1, keepdims=True)
        t[...] = c
        rs = jax.lax.rsqrt(jnp.mean(c * c, axis=-1, keepdims=True) + EPS)
        return jnp.concatenate([t[0:8, :], t[8:16, :]], axis=0) * rs

    def ln_stage(k, ln, slots=True):
        RB = LN_RB
        lnf = ln_slot if slots else (lambda v, slot: _layernorm(v))
        for r in range(TM // RB):
            pr = slice(r * RB // 2, (r + 1) * RB // 2)
            gr = prow(k, RB // 2, r * RB // 2)
            xn = lnf(upk(x_v[gr, :]).astype(f32), (2 * r) % NSLOT).astype(bf16)
            xn_v[gr, :] = pk(xn)
            ln[0][pr, :] = pk(xn)
            ln[1][pr, :] = pk(lnf(xn.astype(f32), (2 * r + 1) % NSLOT).astype(bf16))
        return ln

    def b_piece(xn, j, wref):
        return jax.lax.dot_general(upk(xn[...]), upk(wref[64 * j:64 * j + 64, :]), _NT_DIMS,
                                   preferred_element_type=f32)

    def to_segments(ref, val):
        for g in range(TM // 8):
            sg, gq = divmod(g, SEG // 8)
            ref[pl.ds(64 * gq + sg, 8, stride=8), :] = val[8 * g:8 * g + 8]

    def from_segments(ref, base):
        parts = []
        for g in range(TM // 8):
            sg, gq = divmod(g, SEG // 8)
            parts.append(ref[pl.ds(base + 64 * gq + sg, 8, stride=8), :])
        return jnp.concatenate(parts, axis=0)

    sub1 = jax.lax.broadcasted_iota(jnp.int32, (8, LANES), 0)

    def scan_piece(j, hr_o, hi_o, par=0):
        ls = tile(j)
        ur, ui = u_ab[par][2 * j], u_ab[par][2 * j + 1]
        l_r = tab_v[11, :, ls]
        l_i = tab_v[12, :, ls]

        def step(hr, hi, m):
            return (l_r * hr - l_i * hi + ur[8 * m:8 * m + 8, :],
                    l_r * hi + l_i * hr + ui[8 * m:8 * m + 8, :])
        er, ei = ur[0:8, :], ui[0:8, :]
        for m in range(1, SEG):
            er, ei = step(er, ei, m)
        for i, d in enumerate((1, 2, 4)):
            a_r = tab_v[2 * i, :, ls]
            a_i = tab_v[2 * i + 1, :, ls]
            sr = pltpu.roll(er, d, 0)
            si = pltpu.roll(ei, d, 0)
            er, ei = er + (a_r * sr - a_i * si), ei + (a_r * si + a_i * sr)
        q_r = tab_v[6, :, ls]
        q_i = tab_v[7, :, ls]
        c_r = carry_v[0, :, ls]
        c_i = carry_v[1, :, ls]
        er, ei = er + (q_r * c_r - q_i * c_i), ei + (q_r * c_i + q_i * c_r)
        carry_v[0, :, ls] = jnp.broadcast_to(er[7:8, :], (8, LANES))
        carry_v[1, :, ls] = jnp.broadcast_to(ei[7:8, :], (8, LANES))
        hr = jnp.where(sub1 == 0, c_r, pltpu.roll(er, 1, 0))
        hi = jnp.where(sub1 == 0, c_i, pltpu.roll(ei, 1, 0))
        f_r = tab_v[8, :, ls]
        f_i = tab_v[9, :, ls]
        for p in range(SEG // 2):
            outs = []
            for m in (2 * p, 2 * p + 1):
                hr, hi = step(hr, hi, m)
                outs.append((f_r * hr - f_i * hi, -(f_r * hi) - f_i * hr))
            hr_o[8 * p:8 * p + 8, ls] = pk(jnp.concatenate([outs[0][0], outs[1][0]], axis=0).astype(bf16))
            hi_o[8 * p:8 * p + 8, ls] = pk(jnp.concatenate([outs[0][1], outs[1][1]], axis=0).astype(bf16))

    def c_piece(k, j, hr_i, hi_i):
        y = jax.lax.dot_general(upk(hr_i[...]), upk(cre_v[64 * j:64 * j + 64, :]), _NT_DIMS,
                                preferred_element_type=f32)
        y = y + jax.lax.dot_general(upk(hi_i[...]), upk(cim_v[64 * j:64 * j + 64, :]), _NT_DIMS,
                                    preferred_element_type=f32)
        y_v[j, rows_of(k), :] = y

    def w_piece(k, xn2, j):
        pre = jnp.dot(upk(xn2[...]), upk(w1_v[:, tile(j)]), preferred_element_type=f32)
        for r in range(TM // 64):
            h1_v[rows_of(k, 64, PAD + 64 * r), tile(j)] = _gelu(pre[64 * r:64 * r + 64])

    def b_step(xn, j, part, par=0):
        to_segments(u_ab[par][2 * j + part], b_piece(xn, j, (bre_v, bim_v)[part]))

    def p1_iter(k, hcur, hprev, ln, lnprev):
        xn, _ = ln_stage(k, ln)
        for kind, j in ORDER:
            if kind == "c":
                c_piece(k - 1, j, *hprev)
            elif kind == "b":
                b_step(xn, j, 0)
                b_step(xn, j, 1)
                scan_piece(j, *hcur)
            else:
                w_piece(k - 1, lnprev[1], j)

    lane = jax.lax.broadcasted_iota(jnp.int32, (TM, LANES), 1)

    def w2_stage(k, x1_o, n3_o):
        def sh(j, s):
            win = h1_v[rows_of(k, TM + 2 * PAD), tile(j)]
            return win[PAD - s:PAD - s + TM]
        g = jnp.concatenate([
            sh(0, 1),
            jnp.where(lane < 32, sh(1, 1), sh(1, -1)),
            jnp.where(lane < 64, sh(2, -1), sh(2, 2)),
            jnp.where(lane < 96, sh(3, 2), sh(3, -2)),
            sh(4, -2)], axis=1).astype(bf16)
        hs = jnp.dot(g, upk(w2_v[...]), preferred_element_type=f32)
        x1 = upk(xn_v[prow(k), :]).astype(f32) + hs
        x1_o[...] = x1
        n3_o[...] = pk(_layernorm(x1).astype(bf16))

    def o_copy(k):
        return pltpu.make_async_copy(o_v.at[rows_of(k), :], o_hbm.at[rows_of(k), :], osem.at[k])

    def o_tile_copy(j):
        return pltpu.make_async_copy(o_v.at[rows_of(NC - 1), tile(j)], o_hbm.at[rows_of(NC - 1), tile(j)],
                                     osem.at[NC + j])

    def mlp_last(k, x1_i, n3_i):
        hid = _gelu(jnp.dot(upk(n3_i[...]), upk(w3_v[...]), preferred_element_type=f32)).astype(bf16)
        for j in range(NT):
            h2 = jnp.dot(hid, upk(w4_v[:, tile(j)]), preferred_element_type=f32)
            gate = _silu(x1_i[:, tile(j)] + h2)
            s = from_segments(y_v.at[j], k * TM) + upk(xn_v[prow(k), tile(j)]).astype(f32) * tab_v[10, 0:1, tile(j)]
            o_v[rows_of(k), tile(j)] = upk(x_v[prow(k), tile(j)]).astype(f32) + s * gate
            o_tile_copy(j).start()

    def mlp_stage(k, x1_i, n3_i, mid):
        pre = jnp.dot(upk(n3_i[...]), upk(w3_v[...]), preferred_element_type=f32)
        mid()
        hid = _gelu(pre).astype(bf16)
        h2 = jnp.dot(hid, upk(w4_v[...]), preferred_element_type=f32)
        gate = _silu(x1_i[...] + h2)
        s = jnp.concatenate([from_segments(y_v.at[j], k * TM) for j in range(NT)], axis=1)
        s = s + upk(xn_v[prow(k), :]).astype(f32) * tab_v[10, 0:1, :]
        o_v[rows_of(k), :] = upk(x_v[prow(k), :]).astype(f32) + s * gate
        o_copy(k).start()

    HS, LS = ((hra, hia), (hrb, hib), hc), (lna, lnb, lnc)
    x_copy(0).wait()
    xn0, _ = ln_stage(0, lna, slots=False)
    bre_a.wait()
    for j in range(NA):
        b_step(xn0, j, 0, 0)
    x_copy(1).wait()
    bre_b.wait()
    xn1, _ = ln_stage(1, lnb, slots=False)
    for j in range(NA, NT):
        b_step(xn0, j, 0, 0)
    for j in range(NT):
        b_step(xn1, j, 0, 1)
    wc["bim"].wait()
    for j in range(NT):
        b_step(xn0, j, 1, 0)
        if j == NT - 1:
            wc["w1"].wait()
        scan_piece(j, *HS[0], par=0)
    for j in range(NT):
        w_piece(0, lna[1], j)
        b_step(xn1, j, 1, 1)
        if j == NT - 1:
            wc["cre"].wait()
            wc["cim"].wait()
        scan_piece(j, *HS[1], par=1)
    for j in range(NT):
        c_piece(0, j, *HS[0])

    def p1_body(q, c):
        k = 3 * q + 2
        for i in range(3):
            x_copy(k + i).wait()
        for i in range(3):
            cur, prev = (2 + i) % 3, (1 + i) % 3
            p1_iter(k + i, HS[cur], HS[prev], LS[cur], LS[prev])
        return c
    jax.lax.fori_loop(0, (NC - 2) // 3, p1_body, 0)

    wc["w2"].wait()
    wc["w3"].wait()
    wc["w4"].wait()
    last = (NC - 1) % 3
    for j in range(NT):
        w_piece(NC - 1, LS[last][1], j)
    w2_stage(0, x1a, n3a)
    for j in range(NT):
        c_piece(NC - 1, j, *HS[last])

    def p2_body(q, c):
        k = 2 * q
        mlp_stage(k, x1a, n3a, lambda: w2_stage(k + 1, x1b, n3b))
        mlp_stage(k + 1, x1b, n3b, lambda: w2_stage(k + 2, x1a, n3a))
        return c
    jax.lax.fori_loop(0, (NC - 2) // 2, p2_body, 0)
    mlp_stage(NC - 2, x1a, n3a, lambda: w2_stage(NC - 1, x1b, n3b))
    mlp_last(NC - 1, x1b, n3b)
    for k in range(NC - 1):
        o_copy(k).wait()
    for j in range(NT):
        o_tile_copy(j).wait()


@jax.jit
def pallas_recurrent_scan__ssm_conv_s5__mixer_s_mlp__prompt_kernel(
    A_x: jax.Array,
    A_Lambda_re: jax.Array,
    A_Lambda_im: jax.Array,
    A_B_re: jax.Array,
    A_B_im: jax.Array,
    A_C_re: jax.Array,
    A_C_im: jax.Array,
    A_log_dt: jax.Array,
    A_Dskip: jax.Array,
    B_x: jax.Array,
    B_w1: jax.Array,
    B_w2: jax.Array,
    B_w3: jax.Array,
    B_w4: jax.Array,
):
    del B_x
    x = A_x.reshape(L, D)
    hbm = pl.BlockSpec(memory_space=pl.ANY)
    out = pl.pallas_call(
        _kernel,
        out_shape=jax.ShapeDtypeStruct((L, D), f32),
        in_specs=[hbm] * 13,
        out_specs=hbm,
        scratch_shapes=[
            pltpu.VMEM((L // 2, D), u32),
            pltpu.VMEM((P // 2, D), u32), pltpu.VMEM((P // 2, D), u32),
            pltpu.VMEM((D // 2, P), u32), pltpu.VMEM((D // 2, P), u32),
            pltpu.VMEM((D // 2, D), u32), pltpu.VMEM((D // 2, D), u32),
            pltpu.VMEM((D // 2, F), u32), pltpu.VMEM((F // 2, D), u32),
            pltpu.VMEM((L // 2, D), u32),
            pltpu.VMEM((L + 2 * PAD, D), f32),
            pltpu.VMEM((NT, L, LANES), f32),
            pltpu.VMEM((L, D), f32),
            pltpu.VMEM((TM // 2, P), u32), pltpu.VMEM((TM // 2, P), u32),
            pltpu.VMEM((TM // 2, P), u32), pltpu.VMEM((TM // 2, P), u32),
            pltpu.VMEM((TM, D), f32), pltpu.VMEM((TM, D), f32),
            pltpu.VMEM((TM // 2, D), u32), pltpu.VMEM((TM // 2, D), u32),
            pltpu.VMEM((13, 8, P), f32),
            pltpu.VMEM((2, 8, P), f32),
            pltpu.VMEM((P,), bf16), pltpu.VMEM((P,), bf16), pltpu.VMEM((P,), bf16), pltpu.VMEM((D,), bf16),
            pltpu.SemaphoreType.DMA((NC,)),
            pltpu.SemaphoreType.DMA((9,)),
            pltpu.SemaphoreType.DMA((NC + NT,)),
            pltpu.SemaphoreType.DMA((4,)),
        ]
        + [pltpu.VMEM((TM, LANES), f32)] * (4 * NT)
        + [pltpu.VMEM((TM // 2, D), u32)] * 4
        + [pltpu.VMEM((NSLOT, LN_RB, D), f32)]
        + [pltpu.VMEM((TM // 2, D), u32)] * 4,
        compiler_params=pltpu.CompilerParams(vmem_limit_bytes=100 * 1024 * 1024),
    )(x, A_Lambda_re, A_Lambda_im, A_B_re, A_B_im, A_C_re, A_C_im, A_log_dt, A_Dskip,
      B_w1, B_w2, B_w3, B_w4)
    return out.reshape(1, L, D)
```
